```python
import os as _os
_os.environ.setdefault("JAX_PLATFORMS", "cpu")
import jax
import jax.numpy as jnp

def _softmax(x, axis=-1):
    return jax.nn.softmax(x, axis=axis)
def _gelu(x):
    return jax.nn.gelu(x, approximate=True)
def _silu(x):
    return jax.nn.silu(x)
def _sigmoid(x):
    return jax.nn.sigmoid(x)
def _layernorm(x, axis=-1, eps=1e-5):
    m = jnp.mean(x, axis=axis, keepdims=True)
    v = jnp.var(x, axis=axis, keepdims=True)
    return (x - m) / jnp.sqrt(v + eps)
def _scatter_add(tgt, idx, src, axis=0):
    return tgt.at[idx].add(src)
def _segment_sum(src, seg, n):
    return jax.ops.segment_sum(src, seg, n)
class _Rng:
    def __init__(self, key):
        self._k = key
    def _next(self):
        self._k, sub = jax.random.split(self._k)
        return sub
    def normal(self, shape):
        return jax.random.normal(self._next(), shape, dtype=jnp.bfloat16)
    def randint(self, lo, hi, shape):
        return jax.random.randint(self._next(), shape, lo, hi, dtype=jnp.int32)
    def uniform(self, shape, lo=0.0, hi=1.0):
        return jax.random.uniform(self._next(), shape, jnp.bfloat16, lo, hi)
    def permutation(self, n):
        return jax.random.permutation(self._next(), n)


kernel_name = 'gated_mix__linear_attn_block__glu_gated_swiglu__prompt'

def setup_inputs():
    _rng = _Rng(jax.random.key(int.from_bytes(__import__("os").urandom(4), "little")))
    _w = (lambda a: (lambda t: t.astype(jnp.bfloat16) if jnp.issubdtype(t.dtype, jnp.floating) else t)(jnp.asarray(a)))
    def _A_setup():
        B, S, D = 1, 2048, 1024
        return {
            "x": _w((lambda *s: _rng.normal(s) * 0.05)(B, S, D)),
            "wqkv": _w((lambda *s: _rng.normal(s) * 0.8)(D, 3 * D)),
            "wo": _w((lambda *s: _rng.normal(s) * 0.05)(D, D)),
        }
    _A_in = _A_setup()

    def _B_setup():
        B, S, D, F = 1, 2048, 1024, 3584
        return {
            "x": _w((lambda *s: _rng.normal(s) * 0.05)(B, S, D)),
            "w1": _w((lambda *s: _rng.normal(s) * 1.6)(D, F) * (2.0 / D) ** 0.5),
            "w3": _w((lambda *s: _rng.normal(s) * 1.6)(D, F) * (2.0 / D) ** 0.5),
            "w2": _w((lambda *s: _rng.normal(s) * 1.6)(F, D) * (2.0 / F) ** 0.5),
        }
    _B_in = _B_setup()

    return {
        "A_x": _A_in["x"],
        "A_wqkv": _A_in["wqkv"],
        "A_wo": _A_in["wo"],
        "B_x": _B_in["x"],
        "B_w1": _B_in["w1"],
        "B_w3": _B_in["w3"],
        "B_w2": _B_in["w2"],
        "gate_w": _w((lambda *s: _rng.normal(s) * 0.05)(1024) * 16.0),
    }

def reference(A_x, A_wqkv, A_wo, B_x, B_w1, B_w3, B_w2, gate_w):
    def _A_ref(x, wqkv, wo):
        B, S, D = x.shape
        H = 32; Dh = D // H
        qkv = (lambda x, *d: x.transpose(*d))((x @ wqkv).reshape(B, S, 3, H, Dh), 2, 0, 3, 1, 4)
        q, k, v = qkv[0], qkv[1], qkv[2]
        phi = lambda t: jnp.where(t > 0, t + 1, jnp.exp(t)) + 1e-6
        pq, pk = phi(q), phi(k)
        kv = jnp.einsum("bhsd,bhse->bhde", pk, v)
        z = jnp.einsum("bhsd->bhd", pk)
        num = jnp.einsum("bhqd,bhde->bhqe", pq, kv)
        den = jnp.einsum("bhqd,bhd->bhq", pq, z)[..., None] + 1e-6
        o = num / den
        return (lambda x, *d: x.transpose(*d))(o, 0, 2, 1, 3).reshape(B, S, D) @ wo

    def _B_ref(x, w1, w3, w2):
        gate = jnp.einsum("bsd,df->bsf", x, w1)
        up = jnp.einsum("bsd,df->bsf", x, w3)
        h = _silu(gate) * up
        out = jnp.einsum("bsf,fd->bsd", h, w2)
        return out

    x = A_x
    g = _sigmoid((x * gate_w).sum(-1, keepdims=True))
    a = _A_ref(x, A_wqkv, A_wo)
    b = _B_ref(x, B_w1, B_w3, B_w2)
    return g * a + (1 - g) * b
```

```python
import functools
import jax
import jax.numpy as jnp
from jax import lax
import jax.experimental.pallas as pl
import jax.experimental.pallas.tpu as pltpu

S, D, F, H = 2048, 1024, 3584, 32
DH = D // H
G = 128
NG = D // G


def _phi(t):
    return jnp.where(t > 0, t + 1.0, jnp.exp(t)) + 1e-6


def _build(tm=256, tm1=512, fc=512, wc=512, scopes=False):
    n = S // tm
    n1 = S // tm1
    nf = F // fc
    nw = D // wc

    SEM_X = 0
    SEM_K = SEM_X + n1
    SEM_V = SEM_K + nw
    SEM_Q = SEM_V + nw
    SEM_O = SEM_Q + 1
    SEM_1 = SEM_O + 1
    SEM_3 = SEM_1 + nf
    SEM_2 = SEM_3 + nf
    SEM_OUT = SEM_2 + nf
    NSEM = SEM_OUT + 2

    def kernel(x_hbm, wqkv_hbm, wo_hbm, w1_hbm, w3_hbm, w2_hbm, gw_ref, o_hbm,
               x_v, wqkv_v, wo_v, w1_v, w3_v, w2_v, m_v, zbd_v, obuf, sems):

        def cp_x(c):
            return pltpu.make_async_copy(x_hbm.at[pl.ds(c * tm1, tm1), :],
                                         x_v.at[pl.ds(c * tm1, tm1), :], sems.at[SEM_X + c])

        def cp_k(c):
            return pltpu.make_async_copy(wqkv_hbm.at[:, pl.ds(D + c * wc, wc)],
                                         wqkv_v.at[:, pl.ds(D + c * wc, wc)], sems.at[SEM_K + c])

        def cp_v(c):
            return pltpu.make_async_copy(wqkv_hbm.at[:, pl.ds(2 * D + c * wc, wc)],
                                         wqkv_v.at[:, pl.ds(2 * D + c * wc, wc)], sems.at[SEM_V + c])

        def cp_q():
            return pltpu.make_async_copy(wqkv_hbm.at[:, pl.ds(0, D)],
                                         wqkv_v.at[:, pl.ds(0, D)], sems.at[SEM_Q])

        def cp_o():
            return pltpu.make_async_copy(wo_hbm, wo_v, sems.at[SEM_O])

        def cp_1(c):
            return pltpu.make_async_copy(w1_hbm.at[:, pl.ds(c * fc, fc)],
                                         w1_v.at[:, pl.ds(c * fc, fc)], sems.at[SEM_1 + c])

        def cp_3(c):
            return pltpu.make_async_copy(w3_hbm.at[:, pl.ds(c * fc, fc)],
                                         w3_v.at[:, pl.ds(c * fc, fc)], sems.at[SEM_3 + c])

        def cp_2(c):
            return pltpu.make_async_copy(w2_hbm.at[pl.ds(c * fc, fc), :],
                                         w2_v.at[pl.ds(c * fc, fc), :], sems.at[SEM_2 + c])

        def cp_out(i, slot):
            r0 = pl.multiple_of(i * tm, tm)
            return pltpu.make_async_copy(obuf.at[slot], o_hbm.at[pl.ds(r0, tm), :], sems.at[SEM_OUT + slot])

        def _phase1():
            cp_x(0).start()
            for c in range(nw):
                cp_k(c).start()
                cp_v(c).start()
            for c in range(1, n1):
                cp_x(c).start()

            kv = [None] * NG
            z = [None] * nw
            for c in range(n1):
                cp_x(c).wait()
                xb = x_v[pl.ds(c * tm1, tm1), :]
                for j in range(nw):
                    if c == 0:
                        cp_k(j).wait()
                        cp_v(j).wait()
                        if j == nw - 1:
                            cp_o().start()
                            cp_q().start()
                            for f in range(nf):
                                cp_1(f).start()
                                cp_3(f).start()
                                cp_2(f).start()
                    k = jnp.dot(xb, wqkv_v[:, pl.ds(D + j * wc, wc)], preferred_element_type=jnp.float32)
                    v = jnp.dot(xb, wqkv_v[:, pl.ds(2 * D + j * wc, wc)], preferred_element_type=jnp.float32)
                    pk = _phi(k)
                    zc = jnp.sum(pk, axis=0, keepdims=True)
                    z[j] = zc if c == 0 else z[j] + zc
                    pkb = pk.astype(jnp.bfloat16)
                    vb = v.astype(jnp.bfloat16)
                    for gg in range(wc // G):
                        g = j * (wc // G) + gg
                        part = lax.dot_general(pkb[:, gg * G:(gg + 1) * G], vb[:, gg * G:(gg + 1) * G],
                                               (((0,), (0,)), ((), ())),
                                               preferred_element_type=jnp.float32)
                        kv[g] = part if c == 0 else kv[g] + part
            cp_o().wait()
            ri = lax.broadcasted_iota(jnp.int32, (G, G), 0) // DH
            ci = lax.broadcasted_iota(jnp.int32, (G, G), 1) // DH
            mask = ri == ci
            for g in range(NG):
                kvm = jnp.where(mask, kv[g], 0.0).astype(jnp.bfloat16)
                m_v[pl.ds(g * G, G), :] = jnp.dot(kvm, wo_v[pl.ds(g * G, G), :],
                                                  preferred_element_type=jnp.float32).astype(jnp.bfloat16)
                j, gg = divmod(g, wc // G)
                zcol = jnp.transpose(jnp.broadcast_to(z[j][:, gg * G:(gg + 1) * G], (G, G)))
                zbd_v[g] = jnp.where(mask, zcol, 0.0).astype(jnp.bfloat16)
            cp_q().wait()
            for f in range(nf):
                cp_1(f).wait()
                cp_3(f).wait()
                cp_2(f).wait()

        def _phase2(i, carry):
            slot = i % 2
            r0 = pl.multiple_of(i * tm, tm)
            xb = x_v[pl.ds(r0, tm), :]
            gl = jnp.sum(xb.astype(jnp.float32) * gw_ref[...].astype(jnp.float32), axis=1, keepdims=True)
            gate = jax.nn.sigmoid(gl)
            q = jnp.dot(xb, wqkv_v[:, pl.ds(0, D)], preferred_element_type=jnp.float32)
            pq = _phi(q)
            pqb = pq.astype(jnp.bfloat16)
            den = jnp.concatenate(
                [jnp.dot(pqb[:, g * G:(g + 1) * G], zbd_v[g], preferred_element_type=jnp.float32)
                 for g in range(NG)], axis=1) + 1e-6
            pqn = (pq / den).astype(jnp.bfloat16)
            a = jnp.dot(pqn, m_v[...], preferred_element_type=jnp.float32)
            b = None
            for f in range(nf):
                gt = jnp.dot(xb, w1_v[:, pl.ds(f * fc, fc)], preferred_element_type=jnp.float32)
                up = jnp.dot(xb, w3_v[:, pl.ds(f * fc, fc)], preferred_element_type=jnp.float32)
                h = (gt * jax.nn.sigmoid(gt) * up).astype(jnp.bfloat16)
                part = jnp.dot(h, w2_v[pl.ds(f * fc, fc), :], preferred_element_type=jnp.float32)
                b = part if b is None else b + part
            res = (gate * a + (1.0 - gate) * b).astype(obuf.dtype)

            @pl.when(i >= 2)
            def _():
                cp_out(i - 2, slot).wait()
            obuf[slot] = res
            cp_out(i, slot).start()
            return carry

        if scopes:
            with jax.named_scope('phase1'):
                _phase1()
            with jax.named_scope('phase2'):
                lax.fori_loop(0, n, _phase2, 0)
        else:
            _phase1()
            lax.fori_loop(0, n, _phase2, 0)
        cp_out(n - 2, (n - 2) % 2).wait()
        cp_out(n - 1, (n - 1) % 2).wait()

    @jax.jit
    def fn(A_x, A_wqkv, A_wo, B_x, B_w1, B_w3, B_w2, gate_w):
        x2 = A_x.reshape(S, D)
        gw = gate_w.reshape(1, D)
        out = pl.pallas_call(
            kernel,
            in_specs=[pl.BlockSpec(memory_space=pl.ANY)] * 6 + [pl.BlockSpec(memory_space=pltpu.VMEM)],
            out_specs=pl.BlockSpec(memory_space=pl.ANY),
            out_shape=jax.ShapeDtypeStruct((S, D), jnp.bfloat16),
            scratch_shapes=[
                pltpu.VMEM((S, D), jnp.bfloat16),
                pltpu.VMEM((D, 3 * D), jnp.bfloat16),
                pltpu.VMEM((D, D), jnp.bfloat16),
                pltpu.VMEM((D, F), jnp.bfloat16),
                pltpu.VMEM((D, F), jnp.bfloat16),
                pltpu.VMEM((F, D), jnp.bfloat16),
                pltpu.VMEM((D, D), jnp.bfloat16),
                pltpu.VMEM((NG, G, G), jnp.bfloat16),
                pltpu.VMEM((2, tm, D), jnp.bfloat16),
                pltpu.SemaphoreType.DMA((NSEM,)),
            ],
            compiler_params=pltpu.CompilerParams(
                vmem_limit_bytes=110 * 1024 * 1024),
        )(x2, A_wqkv, A_wo, B_w1, B_w3, B_w2, gw)
        return out.reshape(1, S, D)
    return fn


_fn = _build()


@jax.jit
def pallas_gated_mix__linear_attn_block__glu_gated_swiglu__prompt_kernel(
    A_x: jax.Array,
    A_wqkv: jax.Array,
    A_wo: jax.Array,
    B_x: jax.Array,
    B_w1: jax.Array,
    B_w3: jax.Array,
    B_w2: jax.Array,
    gate_w: jax.Array,
):
    return _fn(A_x, A_wqkv, A_wo, B_x, B_w1, B_w3, B_w2, gate_w)
```

```python
import jax
import jax.numpy as jnp
from jax import lax
import jax.experimental.pallas as pl
import jax.experimental.pallas.tpu as pltpu

S, D, F, H = 2048, 1024, 3584, 32
DH = D // H
G = 128
NG = D // G

TM = 256
TM1 = 256
FC = 512
WC = 512
TSPLIT = 2

N = S // TM
N1 = S // TM1
NF = F // FC
NW = D // WC

SEM_X = 0
SEM_K = SEM_X + N1
SEM_V = SEM_K + NW
SEM_Q = SEM_V + NW
SEM_O = SEM_Q + 1
SEM_1 = SEM_O + 1
SEM_3 = SEM_1 + NF
SEM_2 = SEM_3 + NF
SEM_OUT = SEM_2 + NF
SEM_G = SEM_OUT + 2
NSEM = SEM_G + 1


def _phi(t):
    return jnp.where(t > 0, t + 1.0, jnp.exp(t)) + 1e-6


def _kernel(x_hbm, wqkv_hbm, wo_hbm, w1_hbm, w3_hbm, w2_hbm, gw_hbm, o_hbm,
            x_v, wqkv_v, wo_v, w1_v, w3_v, w2_v, m_v, obuf, kv_v, z_v, gw_v, sems):

    def cp_x(c):
        r0 = c * TM1 if isinstance(c, int) else pl.multiple_of(c * TM1, TM1)
        return pltpu.make_async_copy(x_hbm.at[pl.ds(r0, TM1), :],
                                     x_v.at[pl.ds(r0, TM1), :], sems.at[SEM_X + c])

    def cp_k(c):
        return pltpu.make_async_copy(wqkv_hbm.at[:, pl.ds(D + c * WC, WC)],
                                     wqkv_v.at[:, pl.ds(D + c * WC, WC)], sems.at[SEM_K + c])

    def cp_v(c):
        return pltpu.make_async_copy(wqkv_hbm.at[:, pl.ds(2 * D + c * WC, WC)],
                                     wqkv_v.at[:, pl.ds(2 * D + c * WC, WC)], sems.at[SEM_V + c])

    def cp_q():
        return pltpu.make_async_copy(wqkv_hbm.at[:, pl.ds(0, D)],
                                     wqkv_v.at[:, pl.ds(0, D)], sems.at[SEM_Q])

    def cp_o():
        return pltpu.make_async_copy(wo_hbm, wo_v, sems.at[SEM_O])

    def cp_1(c):
        return pltpu.make_async_copy(w1_hbm.at[:, pl.ds(c * FC, FC)],
                                     w1_v.at[:, pl.ds(c * FC, FC)], sems.at[SEM_1 + c])

    def cp_3(c):
        return pltpu.make_async_copy(w3_hbm.at[:, pl.ds(c * FC, FC)],
                                     w3_v.at[:, pl.ds(c * FC, FC)], sems.at[SEM_3 + c])

    def cp_2(c):
        return pltpu.make_async_copy(w2_hbm.at[pl.ds(c * FC, FC), :],
                                     w2_v.at[pl.ds(c * FC, FC), :], sems.at[SEM_2 + c])

    def cp_g():
        return pltpu.make_async_copy(gw_hbm, gw_v.at[pl.ds(0, D)], sems.at[SEM_G])

    def cp_out(i, slot):
        r0 = pl.multiple_of(i * TM, TM)
        return pltpu.make_async_copy(obuf.at[slot], o_hbm.at[pl.ds(r0, TM), :],
                                     sems.at[SEM_OUT + slot])

    def start_big():
        cp_q().start()
        cp_o().start()
        cp_g().start()
        for f in range(NF):
            cp_1(f).start()
            cp_3(f).start()
            cp_2(f).start()

    def p1_chunk(c, first):
        cp_x(c).wait()
        r0 = c * TM1 if isinstance(c, int) else pl.multiple_of(c * TM1, TM1)
        xb = x_v[pl.ds(r0, TM1), :]
        for j in range(NW):
            if first:
                cp_k(j).wait()
            k = jnp.dot(xb, wqkv_v[:, pl.ds(D + j * WC, WC)], preferred_element_type=jnp.float32)
            if first:
                cp_v(j).wait()
                if j == NW - 1:
                    start_big()
            v = jnp.dot(xb, wqkv_v[:, pl.ds(2 * D + j * WC, WC)], preferred_element_type=jnp.float32)
            pk = _phi(k)
            zc = jnp.sum(pk, axis=0, keepdims=True)
            if first:
                z_v[:, pl.ds(j * WC, WC)] = zc
            else:
                z_v[:, pl.ds(j * WC, WC)] += zc
            pkb = pk.astype(jnp.bfloat16)
            vb = v.astype(jnp.bfloat16)
            for gg in range(WC // G):
                g = j * (WC // G) + gg
                part = lax.dot_general(pkb[:, gg * G:(gg + 1) * G], vb[:, gg * G:(gg + 1) * G],
                                       (((0,), (0,)), ((), ())),
                                       preferred_element_type=jnp.float32)
                if first:
                    kv_v[g] = part
                else:
                    kv_v[g] += part

    cp_x(0).start()
    for c in range(NW):
        cp_k(c).start()
        cp_v(c).start()
    for c in range(1, N1):
        cp_x(c).start()
    p1_chunk(0, True)

    def p1_body(c, carry):
        p1_chunk(c, False)
        return carry
    lax.fori_loop(1, N1, p1_body, 0)

    cp_o().wait()
    ri = lax.broadcasted_iota(jnp.int32, (G, G), 0) // DH
    ci = lax.broadcasted_iota(jnp.int32, (G, G), 1) // DH
    mask = ri == ci
    for g in range(NG):
        kvm = jnp.where(mask, kv_v[g], 0.0).astype(jnp.bfloat16)
        m_v[pl.ds(g * G, G), :] = jnp.dot(kvm, wo_v[pl.ds(g * G, G), :],
                                          preferred_element_type=jnp.float32).astype(jnp.bfloat16)
    cp_q().wait()
    cp_g().wait()
    for f in range(NF):
        cp_1(f).wait()
        cp_3(f).wait()
        cp_2(f).wait()

    def p2_body(i, carry):
        slot = i % 2

        @pl.when(i >= 2)
        def _():
            cp_out(i - 2, slot).wait()
        r0 = pl.multiple_of(i * TM, TM)
        xb = x_v[pl.ds(r0, TM), :]
        gw = gw_v[pl.ds(0, D)].astype(jnp.float32).reshape(1, D)
        gl = jnp.sum(xb.astype(jnp.float32) * gw, axis=1, keepdims=True)
        gate = jax.nn.sigmoid(gl)
        omg = 1.0 - gate

        def gu(f):
            gt = jnp.dot(xb, w1_v[:, pl.ds(f * FC, FC)], preferred_element_type=jnp.float32)
            up = jnp.dot(xb, w3_v[:, pl.ds(f * FC, FC)], preferred_element_type=jnp.float32)
            return (gt * jax.nn.sigmoid(gt) * up * omg).astype(jnp.bfloat16)

        def dn(h, f):
            return jnp.dot(h, w2_v[pl.ds(f * FC, FC), :], preferred_element_type=jnp.float32)

        q = jnp.dot(xb, wqkv_v[:, pl.ds(0, D)], preferred_element_type=jnp.float32)
        pq = _phi(q)
        h = gu(0)
        lane = lax.broadcasted_iota(jnp.int32, (TM, G), 1) % DH
        dens = []
        for g in range(NG):
            t = pq[:, g * G:(g + 1) * G] * z_v[:, pl.ds(g * G, G)]
            sh = 1
            while sh < DH:
                t = t + jnp.where(lane >= sh, pltpu.roll(t, sh, 1), pltpu.roll(t, G + sh - DH, 1))
                sh *= 2
            dens.append(t)
        den = jnp.concatenate(dens, axis=1) + 1e-6
        r = pl.reciprocal(den, approx=True)
        r = r * (2.0 - den * r)
        pqn = (pq * (r * gate)).astype(jnp.bfloat16)
        acc = None
        for f in range(1, NF):
            hn = gu(f)
            part = dn(h, f - 1)
            acc = part if acc is None else acc + part
            h = hn
        acc = acc + jnp.dot(pqn, m_v[...], preferred_element_type=jnp.float32)
        cw = D // TSPLIT
        for t in range(TSPLIT):
            last = jnp.dot(h, w2_v[pl.ds((NF - 1) * FC, FC), pl.ds(t * cw, cw)],
                           preferred_element_type=jnp.float32)
            obuf[slot, :, pl.ds(t * cw, cw)] = (acc[:, t * cw:(t + 1) * cw] + last).astype(obuf.dtype)
        cp_out(i, slot).start()
        return carry

    lax.fori_loop(0, N, p2_body, 0)
    cp_out(N - 2, (N - 2) % 2).wait()
    cp_out(N - 1, (N - 1) % 2).wait()


@jax.jit
def pallas_gated_mix__linear_attn_block__glu_gated_swiglu__prompt_kernel(
    A_x: jax.Array,
    A_wqkv: jax.Array,
    A_wo: jax.Array,
    B_x: jax.Array,
    B_w1: jax.Array,
    B_w3: jax.Array,
    B_w2: jax.Array,
    gate_w: jax.Array,
):
    x2 = A_x.reshape(S, D)
    out = pl.pallas_call(
        _kernel,
        in_specs=[pl.BlockSpec(memory_space=pl.ANY)] * 7,
        out_specs=pl.BlockSpec(memory_space=pl.ANY),
        out_shape=jax.ShapeDtypeStruct((S, D), jnp.bfloat16),
        scratch_shapes=[
            pltpu.VMEM((S, D), jnp.bfloat16),
            pltpu.VMEM((D, 3 * D), jnp.bfloat16),
            pltpu.VMEM((D, D), jnp.bfloat16),
            pltpu.VMEM((D, F), jnp.bfloat16),
            pltpu.VMEM((D, F), jnp.bfloat16),
            pltpu.VMEM((F, D), jnp.bfloat16),
            pltpu.VMEM((D, D), jnp.bfloat16),
            pltpu.VMEM((2, TM, D), jnp.bfloat16),
            pltpu.VMEM((NG, G, G), jnp.float32),
            pltpu.VMEM((1, D), jnp.float32),
            pltpu.VMEM((2 * D,), jnp.bfloat16),
            pltpu.SemaphoreType.DMA((NSEM,)),
        ],
        compiler_params=pltpu.CompilerParams(vmem_limit_bytes=110 * 1024 * 1024),
    )(x2, A_wqkv, A_wo, B_w1, B_w3, B_w2, gate_w)
    return out.reshape(1, S, D)
```

```python
import jax
import jax.numpy as jnp
from jax import lax
import jax.experimental.pallas as pl
import jax.experimental.pallas.tpu as pltpu

S, D, F, H = 2048, 1024, 3584, 32
DH = D // H
G = 128
NG = D // G

TM = 256
TM1 = 256
FC = 512
WC = 512
RS = 2
RH = TM // RS

N = S // TM
N1 = S // TM1
NF = F // FC
NW = D // WC

SEM_X = 0
SEM_K = SEM_X + N1
SEM_V = SEM_K + NW
SEM_Q = SEM_V + NW
SEM_O = SEM_Q + 1
SEM_1 = SEM_O + 1
SEM_3 = SEM_1 + 1
SEM_2 = SEM_3 + 1
SEM_OUT = SEM_2 + 1
SEM_G = SEM_OUT + 2 * RS
NSEM = SEM_G + 1


def _phi(t):
    return jnp.where(t > 0, t + 1.0, jnp.exp(t)) + 1e-6


def _kernel(x_hbm, wqkv_hbm, wo_hbm, w1_hbm, w3_hbm, w2_hbm, gw_hbm, o_hbm,
            x_v, wqkv_v, wo_v, w1_v, w3_v, w2_v, m_v, obuf, kv_v, z_v, gw_v, sems):

    def cp_x(c):
        r0 = c * TM1 if isinstance(c, int) else pl.multiple_of(c * TM1, TM1)
        return pltpu.make_async_copy(x_hbm.at[pl.ds(r0, TM1), :],
                                     x_v.at[pl.ds(r0, TM1), :], sems.at[SEM_X + c])

    def cp_k(c):
        return pltpu.make_async_copy(wqkv_hbm.at[:, pl.ds(D + c * WC, WC)],
                                     wqkv_v.at[:, pl.ds(D + c * WC, WC)], sems.at[SEM_K + c])

    def cp_v(c):
        return pltpu.make_async_copy(wqkv_hbm.at[:, pl.ds(2 * D + c * WC, WC)],
                                     wqkv_v.at[:, pl.ds(2 * D + c * WC, WC)], sems.at[SEM_V + c])

    def cp_q():
        return pltpu.make_async_copy(wqkv_hbm.at[:, pl.ds(0, D)],
                                     wqkv_v.at[:, pl.ds(0, D)], sems.at[SEM_Q])

    def cp_o():
        return pltpu.make_async_copy(wo_hbm, wo_v, sems.at[SEM_O])

    def cp_1():
        return pltpu.make_async_copy(w1_hbm, w1_v, sems.at[SEM_1])

    def cp_3():
        return pltpu.make_async_copy(w3_hbm, w3_v, sems.at[SEM_3])

    def cp_2():
        return pltpu.make_async_copy(w2_hbm, w2_v, sems.at[SEM_2])

    def cp_g():
        return pltpu.make_async_copy(gw_hbm, gw_v.at[pl.ds(0, D)], sems.at[SEM_G])

    def cp_out(i, slot, t):
        r0 = pl.multiple_of(i * TM + t * RH, RH)
        return pltpu.make_async_copy(obuf.at[slot, pl.ds(t * RH, RH), :],
                                     o_hbm.at[pl.ds(r0, RH), :],
                                     sems.at[SEM_OUT + slot * RS + t])

    def start_big():
        cp_q().start()
        cp_o().start()
        cp_g().start()
        cp_1().start()
        cp_3().start()
        cp_2().start()

    def p1_chunk(c, first):
        cp_x(c).wait()
        r0 = c * TM1 if isinstance(c, int) else pl.multiple_of(c * TM1, TM1)
        xb = x_v[pl.ds(r0, TM1), :]
        for j in range(NW):
            if first:
                cp_k(j).wait()
            k = jnp.dot(xb, wqkv_v[:, pl.ds(D + j * WC, WC)], preferred_element_type=jnp.float32)
            if first:
                cp_v(j).wait()
                if j == NW - 1:
                    start_big()
            v = jnp.dot(xb, wqkv_v[:, pl.ds(2 * D + j * WC, WC)], preferred_element_type=jnp.float32)
            pk = _phi(k)
            zc = jnp.sum(pk, axis=0, keepdims=True)
            if first:
                z_v[:, pl.ds(j * WC, WC)] = zc
            else:
                z_v[:, pl.ds(j * WC, WC)] += zc
            pkb = pk.astype(jnp.bfloat16)
            vb = v.astype(jnp.bfloat16)
            for gg in range(WC // G):
                g = j * (WC // G) + gg
                part = lax.dot_general(pkb[:, gg * G:(gg + 1) * G], vb[:, gg * G:(gg + 1) * G],
                                       (((0,), (0,)), ((), ())),
                                       preferred_element_type=jnp.float32)
                if first:
                    kv_v[g] = part
                else:
                    kv_v[g] += part

    cp_x(0).start()
    for c in range(NW):
        cp_k(c).start()
        cp_v(c).start()
    for c in range(1, N1):
        cp_x(c).start()
    p1_chunk(0, True)

    def p1_body(c, carry):
        p1_chunk(c, False)
        return carry
    lax.fori_loop(1, N1, p1_body, 0)

    cp_o().wait()
    ri = lax.broadcasted_iota(jnp.int32, (G, G), 0) // DH
    ci = lax.broadcasted_iota(jnp.int32, (G, G), 1) // DH
    mask = ri == ci
    for g in range(NG):
        kvm = jnp.where(mask, kv_v[g], 0.0).astype(jnp.bfloat16)
        m_v[pl.ds(g * G, G), :] = jnp.dot(kvm, wo_v[pl.ds(g * G, G), :],
                                          preferred_element_type=jnp.float32).astype(jnp.bfloat16)
    cp_q().wait()
    cp_g().wait()
    cp_1().wait()
    cp_3().wait()
    cp_2().wait()

    def p2_body(i, carry):
        slot = i % 2

        @pl.when(i >= 2)
        def _():
            for t in range(RS):
                cp_out(i - 2, slot, t).wait()
        r0 = pl.multiple_of(i * TM, TM)
        xb = x_v[pl.ds(r0, TM), :]
        gw = gw_v[pl.ds(0, D)].astype(jnp.float32).reshape(1, D)
        gl = jnp.sum(xb.astype(jnp.float32) * gw, axis=1, keepdims=True)
        gate = jax.nn.sigmoid(gl)
        omg = 1.0 - gate

        def gu(f):
            gt = jnp.dot(xb, w1_v[:, pl.ds(f * FC, FC)], preferred_element_type=jnp.float32)
            up = jnp.dot(xb, w3_v[:, pl.ds(f * FC, FC)], preferred_element_type=jnp.float32)
            return (gt * jax.nn.sigmoid(gt) * up * omg).astype(jnp.bfloat16)

        def dn(h, f):
            return jnp.dot(h, w2_v[pl.ds(f * FC, FC), :], preferred_element_type=jnp.float32)

        q = jnp.dot(xb, wqkv_v[:, pl.ds(0, D)], preferred_element_type=jnp.float32)
        pq = _phi(q)
        h = gu(0)
        lane = lax.broadcasted_iota(jnp.int32, (TM, G), 1) % DH
        dens = []
        for g in range(NG):
            t = pq[:, g * G:(g + 1) * G] * z_v[:, pl.ds(g * G, G)]
            sh = 1
            while sh < DH:
                t = t + jnp.where(lane >= sh, pltpu.roll(t, sh, 1), pltpu.roll(t, G + sh - DH, 1))
                sh *= 2
            dens.append(t)
        den = jnp.concatenate(dens, axis=1) + 1e-6
        r = pl.reciprocal(den, approx=True)
        r = r * (2.0 - den * r)
        pqn = (pq * (r * gate)).astype(jnp.bfloat16)
        acc = None
        for f in range(1, NF):
            hn = gu(f)
            part = dn(h, f - 1)
            acc = part if acc is None else acc + part
            h = hn
        acc = acc + jnp.dot(pqn, m_v[...], preferred_element_type=jnp.float32)
        for t in range(RS):
            last = jnp.dot(h[t * RH:(t + 1) * RH, :], w2_v[pl.ds((NF - 1) * FC, FC), :],
                           preferred_element_type=jnp.float32)
            obuf[slot, pl.ds(t * RH, RH), :] = (acc[t * RH:(t + 1) * RH, :] + last).astype(obuf.dtype)
            cp_out(i, slot, t).start()
        return carry

    lax.fori_loop(0, N, p2_body, 0)
    for t in range(RS):
        cp_out(N - 2, (N - 2) % 2, t).wait()
        cp_out(N - 1, (N - 1) % 2, t).wait()


@jax.jit
def pallas_gated_mix__linear_attn_block__glu_gated_swiglu__prompt_kernel(
    A_x: jax.Array,
    A_wqkv: jax.Array,
    A_wo: jax.Array,
    B_x: jax.Array,
    B_w1: jax.Array,
    B_w3: jax.Array,
    B_w2: jax.Array,
    gate_w: jax.Array,
):
    x2 = A_x.reshape(S, D)
    out = pl.pallas_call(
        _kernel,
        in_specs=[pl.BlockSpec(memory_space=pl.ANY)] * 7,
        out_specs=pl.BlockSpec(memory_space=pl.ANY),
        out_shape=jax.ShapeDtypeStruct((S, D), jnp.bfloat16),
        scratch_shapes=[
            pltpu.VMEM((S, D), jnp.bfloat16),
            pltpu.VMEM((D, 3 * D), jnp.bfloat16),
            pltpu.VMEM((D, D), jnp.bfloat16),
            pltpu.VMEM((D, F), jnp.bfloat16),
            pltpu.VMEM((D, F), jnp.bfloat16),
            pltpu.VMEM((F, D), jnp.bfloat16),
            pltpu.VMEM((D, D), jnp.bfloat16),
            pltpu.VMEM((2, TM, D), jnp.bfloat16),
            pltpu.VMEM((NG, G, G), jnp.float32),
            pltpu.VMEM((1, D), jnp.float32),
            pltpu.VMEM((2 * D,), jnp.bfloat16),
            pltpu.SemaphoreType.DMA((NSEM,)),
        ],
        compiler_params=pltpu.CompilerParams(vmem_limit_bytes=110 * 1024 * 1024),
    )(x2, A_wqkv, A_wo, B_w1, B_w3, B_w2, gate_w)
    return out.reshape(1, S, D)
```
